```python
import jax
import jax.numpy as jnp

def _softmax(x, axis=-1):
    return jax.nn.softmax(x, axis=axis)
def _gelu(x):
    return jax.nn.gelu(x, approximate=True)
def _silu(x):
    return jax.nn.silu(x)
def _sigmoid(x):
    return jax.nn.sigmoid(x)
def _layernorm(x, axis=-1, eps=1e-5):
    m = jnp.mean(x, axis=axis, keepdims=True)
    v = jnp.var(x, axis=axis, keepdims=True)
    return (x - m) / jnp.sqrt(v + eps)
def _scatter_add(tgt, idx, src, axis=0):
    return tgt.at[idx].add(src)
def _segment_sum(src, seg, n):
    return jax.ops.segment_sum(src, seg, n)
class _Rng:
    def __init__(self, key):
        self._k = key
    def _next(self):
        self._k, sub = jax.random.split(self._k)
        return sub
    def normal(self, shape):
        return jax.random.normal(self._next(), shape, dtype=jnp.bfloat16)
    def randint(self, lo, hi, shape):
        return jax.random.randint(self._next(), shape, lo, hi, dtype=jnp.int32)
    def uniform(self, shape, lo=0.0, hi=1.0):
        return jax.random.uniform(self._next(), shape, jnp.bfloat16, lo, hi)
    def permutation(self, n):
        return jax.random.permutation(self._next(), n)


kernel_name = 'sequential_preLN__grouped_kv_mqa__glu_gated_swiglu__prompt'

def _fwd_setup_inputs():
    _rng = _Rng(jax.random.key(int.from_bytes(__import__("os").urandom(4), "little")))
    _w = (lambda a: (lambda t: t.astype(jnp.bfloat16) if jnp.issubdtype(t.dtype, jnp.floating) else t)(jnp.asarray(a)))
    def _A_setup():
        B, S, D, H = 1, 2048, 512, 32
        Dh = D // H
        return {
            "x": _w((lambda *s: _rng.normal(s) * 0.05)(B, S, D)),
            "wq": _w((lambda *s: _rng.normal(s) * 0.05)(D, H * Dh)),
            "wk": _w((lambda *s: _rng.normal(s) * 0.05)(D, Dh)),
            "wv": _w((lambda *s: _rng.normal(s) * 0.05)(D, Dh)),
            "wo": _w((lambda *s: _rng.normal(s) * 0.05)(H * Dh, D)),
        }
    _A_in = _A_setup()

    def _B_setup():
        B, S, D, F = 1, 2048, 512, 1376
        return {
            "x": _w((lambda *s: _rng.normal(s) * 0.05)(B, S, D)),
            "w1": _w((lambda *s: _rng.normal(s) * 0.05)(D, F) * (2.0 / D) ** 0.5),
            "w3": _w((lambda *s: _rng.normal(s) * 0.05)(D, F) * (2.0 / D) ** 0.5),
            "w2": _w((lambda *s: _rng.normal(s) * 0.05)(F, D) * (2.0 / F) ** 0.5),
        }
    _B_in = _B_setup()

    return {
        "A_x": _A_in["x"],
        "A_wq": _A_in["wq"],
        "A_wk": _A_in["wk"],
        "A_wv": _A_in["wv"],
        "A_wo": _A_in["wo"],
        "B_x": _B_in["x"],
        "B_w1": _B_in["w1"],
        "B_w3": _B_in["w3"],
        "B_w2": _B_in["w2"],
    }

def _fwd_reference(A_x, A_wq, A_wk, A_wv, A_wo, B_x, B_w1, B_w3, B_w2):
    def _A_ref(x, wq, wk, wv, wo):
        B, S, D = x.shape
        H = 32
        Dh = D // H
        q = (lambda x, *d: x.transpose(*d))((x @ wq).reshape(B, S, H, Dh), 0, 2, 1, 3)
        k = x @ wk
        v = x @ wv
        scores = jnp.einsum("bhqd,bkd->bhqk", q, k) * (Dh ** -0.5)
        p = _softmax(scores, axis=-1)
        o = jnp.einsum("bhqk,bkd->bhqd", p, v)
        return (lambda x, *d: x.transpose(*d))(o, 0, 2, 1, 3).reshape(B, S, H * Dh) @ wo

    def _B_ref(x, w1, w3, w2):
        gate = jnp.einsum("bsd,df->bsf", x, w1)
        up = jnp.einsum("bsd,df->bsf", x, w3)
        h = _silu(gate) * up
        out = jnp.einsum("bsf,fd->bsd", h, w2)
        return out

    x = A_x
    h = x + _A_ref(_layernorm(x, axis=-1), A_wq, A_wk, A_wv, A_wo)
    h2 = h + _B_ref(_layernorm(h, axis=-1), B_w1, B_w3, B_w2)
    return h2


def setup_inputs():
    _inp = _fwd_setup_inputs()
    _gk = jax.random.fold_in(jax.random.key(int.from_bytes(__import__("os").urandom(4), "little")), 2**31 - 1)
    _shapes = [[1, 2048, 512]]
    _dtypes = ['bfloat16']
    _gks = jax.random.split(_gk, len(_shapes))
    _gs = [jax.random.normal(k, s, dtype=jnp.dtype(d)) * 0.05 for k, s, d in zip(_gks, _shapes, _dtypes)]
    _inp["grad_out"] = _gs[0]
    return _inp

def reference(A_x, A_wq, A_wk, A_wv, A_wo, B_w1, B_w3, B_w2, B_x, grad_out):
    _const = dict(B_x=B_x)
    def _f(*_d):
        return _fwd_reference(**{'A_x': _d[0], 'A_wq': _d[1], 'A_wk': _d[2], 'A_wv': _d[3], 'A_wo': _d[4], 'B_w1': _d[5], 'B_w3': _d[6], 'B_w2': _d[7], **_const})
    _out, _vjp = jax.vjp(_f, A_x, A_wq, A_wk, A_wv, A_wo, B_w1, B_w3, B_w2)
    _grads = _vjp(grad_out)
    _out0 = jnp.asarray(_out)
    return (_out0, *[jnp.asarray(_g) for _g in _grads])
```

```python
import functools
import math

import jax
import jax.numpy as jnp
import numpy as np
from jax import lax
import jax.experimental.pallas as pl
import jax.experimental.pallas.tpu as pltpu

f32, bf16, i32 = jnp.float32, jnp.bfloat16, jnp.int32

import os as _os
_e = _os.environ.get
UNROLL_F = int(_e('UF', '4'))
UNROLL_B = int(_e('UB', '4'))
LAG_F = int(_e('LAGF', '1'))
LAG_B = int(_e('LAGB', '3'))
KC_F = int(_e('KCF', '256'))
KC_B = int(_e('KCB', '128'))
S, D, H, DH, F = 2048, 512, 32, 16, 1376
BQ = 256
NB = S // BQ
NT_Q = BQ // 128
NO = NB
NU = NT_Q * H
GH = int(_e('GH', '4'))
AUG = 32
F_CHUNKS = ((0, 352), (352, 352), (704, 352), (1056, 320))
EPS = 1e-5
SCALE = DH ** -0.5
LOG2E = 1.4426950408889634
LN2 = 0.6931471805599453
L_MIN = 2.0 ** -60

NT_DIMS = (((1,), (1,)), ((), ()))


def _mm(a, b):
    return jnp.dot(a, b, preferred_element_type=f32)


def _mm_nt(a, b):
    return lax.dot_general(a, b, NT_DIMS, preferred_element_type=f32)


def _pack_rows(x):
    n = x.shape[0]
    x4 = x.reshape(n // 16, 2, 8, 128)
    a = x4[:, 0].reshape(n // 2, 128)
    b = x4[:, 1].reshape(n // 2, 128)
    return pltpu.pack_elementwise([a, b], packed_dtype=bf16)


def _halves(x):
    n = x.shape[0]
    x4 = x.reshape(n // 16, 2, 8, 128)
    return x4[:, 0].reshape(n // 2, 128), x4[:, 1].reshape(n // 2, 128)


def _unpack(x, idx):
    return pltpu.unpack_elementwise(x, index=idx, packed_dtype=bf16, unpacked_dtype=f32)


def _split3(x):
    hi = x.astype(bf16).astype(f32)
    r = x - hi
    mid = r.astype(bf16).astype(f32)
    lo = (r - mid).astype(bf16).astype(f32)
    return hi, mid, lo


def _ln_stats(xt):
    mean = jnp.mean(xt, axis=0, keepdims=True)
    xc = xt - mean
    var = jnp.mean(xc * xc, axis=0, keepdims=True)
    rstd = lax.rsqrt(var + EPS)
    return xc * rstd, rstd


def _ln_bwd(dy, xhat, rstd):
    m1 = jnp.mean(dy, axis=0, keepdims=True)
    m2 = jnp.mean(dy * xhat, axis=0, keepdims=True)
    return rstd * (dy - m1 - xhat * m2)


def _kernel(x_hbm, wq_hbm, wkT_hbm, wvT_hbm, wo_hbm, w1T_hbm, w3T_hbm, w2_hbm, g_hbm,
            out_hbm, dx_hbm, dwq_hbm, dwkT_hbm, dwvT_hbm, dwo_hbm, dw1T_hbm, dw3T_hbm, dw2_hbm,
            x_v, g_v, wq_v, wo_v, w1_v, w3_v, w2_v, wkvT,
            wqT, woT, w1T, w3T, w2T, wkv_v,
            xT_s, xnT_s, mean_s, rstd_s,
            kvrow_s, kaug, vaug, kT, vT, kmax_s,
            qaug, doaug, p_s, o_s, linv_s, t_s, ds_s,
            hhT, dgT, duT,
            dkv_s, dh_s, dxq_s,
            dwq_a, dwo_a, dw1_a, dw3_a, dw2_a,
            out_st, dwq_st, dwo_st, dw1_st, dw3_st, dw2_st, dwkv_st,
            flag_s, in_sem, x_sem, out_sem, dx_sem):

    def x_copy(b):
        rows = pl.ds(pl.multiple_of(b * BQ, BQ), BQ)
        return pltpu.make_async_copy(x_hbm.at[rows, :], x_v.at[rows, :], x_sem.at[b])

    ins = [(wq_hbm, wq_v), (wkT_hbm, wkvT.at[0:DH]), (wvT_hbm, wkvT.at[DH:2 * DH]),
           (wo_hbm, wo_v), (w1T_hbm, w1T), (w3T_hbm, w3T), (w2_hbm, w2_v), (g_hbm, g_v)]
    in_cp = [None] + [pltpu.make_async_copy(s, d, in_sem.at[i]) for i, (s, d) in enumerate(ins)]
    in_cp[2].start()
    in_cp[3].start()
    for b in range(NB):
        x_copy(b).start()
    in_cp[1].start()

    for acc in (dwq_a, dwo_a, dw1_a, dw3_a, dw2_a, dkv_s):
        acc[...] = jnp.zeros(acc.shape, f32)
    flag_s[0] = 0

    in_cp[2].wait()
    in_cp[3].wait()

    wkv_pad = jnp.concatenate([wkvT[...].astype(f32), jnp.zeros((128 - 2 * DH, D), f32)], axis=0)
    wkv_v[...] = wkv_pad.T[:, 0:2 * DH].astype(bf16)

    def setup_blk(b, kn2max):
        r0 = pl.multiple_of(b * BQ, BQ)
        x_copy(b).wait()
        xtb = x_v[pl.ds(r0, BQ), :].T
        xt = xtb.astype(f32)
        mean = jnp.mean(xt, axis=0, keepdims=True)
        xc = xt - mean
        var = jnp.mean(xc * xc, axis=0, keepdims=True)
        rstd = lax.rsqrt(var + EPS)
        xn = (xc * rstd).astype(bf16)
        for t in range(NT_Q):
            sl = slice(t * 128, (t + 1) * 128)
            xT_s[b, t] = xtb[:, sl]
            xnT_s[b, t] = xn[:, sl]
            mean_s[b, t] = jnp.broadcast_to(mean[:, sl], (8, 128))
            rstd_s[b, t] = jnp.broadcast_to(rstd[:, sl], (8, 128))
        kvt = _mm(wkvT[...], xn).astype(bf16)
        kT[b] = kvt[0:DH]
        ones = jnp.ones((DH, BQ), bf16)
        vT[b] = kvt[DH:2 * DH]
        kf = kvt[0:DH].astype(f32)
        kn2 = jnp.sum(kf * kf, axis=0, keepdims=True)
        kvpad = jnp.concatenate([kvt.astype(f32), jnp.zeros((128 - 2 * DH, BQ), f32)], axis=0)
        kvrow_s[pl.ds(r0, BQ), :] = kvpad.T
        del ones
        return jnp.maximum(kn2max, kn2)

    kn2max = lax.fori_loop(0, NB, setup_blk, jnp.zeros((1, BQ), f32))
    kmax = jnp.sqrt(jnp.max(kn2max, axis=1, keepdims=True))
    kmax_s[...] = jnp.broadcast_to(kmax, (8, 128))

    lane = lax.broadcasted_iota(i32, (128, 128), 1)

    def perm_blk(c, _):
        r0 = pl.multiple_of(c * 256, 256)
        ev = kvrow_s[pl.ds(r0, 128, stride=2), :]
        od = kvrow_s[pl.ds(r0 + 1, 128, stride=2), :]
        for half, src in ((0, ev), (1, od)):
            ka = jnp.where(lane < DH, src, jnp.where(lane < DH + 3, 1.0, 0.0))
            vs = pltpu.roll(src, 128 - DH, 1)
            va = jnp.where(lane < DH, vs, jnp.where(lane < DH + 3, 1.0, 0.0))
            ka3 = ka.reshape(16, 8, 128)
            va3 = va.reshape(16, 8, 128)
            for i in range(16):
                rr = pl.multiple_of(r0 + 16 * i + 8 * half, 8)
                t_s[0, pl.ds(16 * i + 8 * half, 8), :] = ka3[i]
                t_s[1, pl.ds(16 * i + 8 * half, 8), :] = va3[i]
            del rr
        kaug[pl.ds(r0, 256), :] = t_s[0, 0:256, 0:AUG].astype(bf16)
        vaug[pl.ds(r0, 256), :] = t_s[1, 0:256, 0:AUG].astype(bf16)
        return _

    lax.fori_loop(0, S // 256, perm_blk, None)

    for i in (4, 5, 6, 7, 8):
        in_cp[i].start()
    in_cp[1].wait()
    wqT[...] = wq_v[...].T

    def prep_ffn_weights():
        in_cp[4].wait()
        woT[...] = wo_v[...].T
        for cp, src, dst in ((in_cp[5], w1T, w1_v), (in_cp[6], w3T, w3_v)):
            cp.wait()
            for (o, n) in ((0, 384), (384, 384), (768, 384), (1152, 224)):
                if n % 128 == 0:
                    dst[:, o:o + n] = src[o:o + n, :].T
                else:
                    blk = jnp.concatenate([src[o:o + n, :], jnp.zeros((256 - n, D), bf16)], axis=0)
                    dst[:, o:o + n] = blk.T[:, 0:n]
        in_cp[7].wait()
        for (o, n) in ((0, 384), (384, 384), (768, 384), (1152, 224)):
            if n % 128 == 0:
                w2T[:, o:o + n] = w2_v[o:o + n, :].T
            else:
                blk = jnp.concatenate([w2_v[o:o + n, :], jnp.zeros((256 - n, D), bf16)], axis=0)
                w2T[:, o:o + n] = blk.T[:, 0:n]
        in_cp[8].wait()

    rows32 = lax.broadcasted_iota(i32, (AUG, 128), 0)

    def attn_fwd():
        nch = S // KC_F
        ngrp = NU // GH

        def scores(g, c):
            kk = kaug[c * KC_F:(c + 1) * KC_F, :]
            return [_mm(kk, qaug[g * GH + j]) for j in range(GH)]

        def exps(g, c, st, ls):
            out = []
            for j in range(GH):
                e = jnp.exp2(st[j])
                out.append(ls[j] + jnp.sum(e.reshape(KC_F // 8, 8, 128), axis=0))
                p_s[g * GH + j, c * KC_F // 2:(c + 1) * KC_F // 2, :] = _pack_rows(e)
            return out

        ls0 = [jnp.zeros((8, 128), f32) for _ in range(GH)]
        for c in range(LAG_F):
            ls0 = exps(0, c, scores(0, c), ls0)

        def group(g, carry):
            ls, lmin = list(carry[0]), carry[1]
            nxt = jnp.minimum(g + 1, ngrp - 1)
            accs = [jnp.zeros((DH, 128), f32) for _ in range(GH)]
            ls_next = [jnp.zeros((8, 128), f32) for _ in range(GH)]
            for c in range(nch):
                cq = c + LAG_F
                wrap = cq >= nch
                tg, cq = (nxt, cq - nch) if wrap else (g, cq)
                st = scores(tg, cq)
                vt = vT[(c * KC_F) // BQ][:, (c * KC_F) % BQ:(c * KC_F) % BQ + KC_F]
                for j in range(GH):
                    p = pltpu.bitcast(p_s[g * GH + j, c * KC_F // 2:(c + 1) * KC_F // 2, :], bf16)
                    accs[j] = accs[j] + _mm(vt, p)
                if wrap:
                    ls_next = exps(tg, cq, st, ls_next)
                else:
                    ls = exps(tg, cq, st, ls)
            for j in range(GH):
                u = g * GH + j
                l = jnp.sum(ls[j], axis=0, keepdims=True)
                linv = 1.0 / l
                o_s[u] = accs[j] * linv
                linv_s[u] = jnp.broadcast_to(linv, (8, 128))
                lmin = jnp.minimum(lmin, l)
            return tuple(ls_next), lmin

        _, lmin = lax.fori_loop(0, ngrp, group, (tuple(ls0), jnp.full((1, 128), jnp.inf, f32)),
                                unroll=UNROLL_F)
        return lmin

    def true_max_fix():
        def unit(u, _):
            q = qaug[u]

            def chunk(c, mx):
                kk = kaug[pl.ds(pl.multiple_of(c * 256, 256), 256), :]
                st = _mm(kk, q)
                return jnp.maximum(mx, jnp.max(st.reshape(32, 8, 128), axis=0))

            mx = lax.fori_loop(0, S // 256, chunk, jnp.full((8, 128), -jnp.inf, f32))
            d = jnp.max(mx, axis=0, keepdims=True)
            qf = q.astype(f32)
            m_old = -(qf[DH:DH + 1] + qf[DH + 1:DH + 2] + qf[DH + 2:DH + 3])
            hi, mid, lo = _split3(-(m_old + d))
            new = jnp.where(rows32 == DH, hi,
                            jnp.where(rows32 == DH + 1, mid,
                                      jnp.where(rows32 == DH + 2, lo, qf)))
            qaug[u] = new.astype(bf16)
            return _

        lax.fori_loop(0, NU, unit, None)

    def attn_bwd():
        nch = S // KC_B
        ngrp = NU // GH

        def dprob(g, c):
            vv = vaug[c * KC_B:(c + 1) * KC_B, :]
            return [_mm(vv, doaug[g * GH + j]) for j in range(GH)]

        def dscore(g, c, dpts):
            for j in range(GH):
                pi = p_s[g * GH + j, c * KC_B // 2:(c + 1) * KC_B // 2, :]
                da, db = _halves(dpts[j])
                ds_s[c % (LAG_B + 1), j] = pltpu.pack_elementwise(
                    [_unpack(pi, 0) * da, _unpack(pi, 1) * db], packed_dtype=bf16)

        for c in range(LAG_B):
            dscore(0, c, dprob(0, c))

        def group(g, _):
            nxt = jnp.minimum(g + 1, ngrp - 1)
            us = [g * GH + j for j in range(GH)]
            dqs = [jnp.zeros((DH, 128), f32) for _ in range(GH)]
            do_cat = jnp.concatenate([doaug[u, 0:DH, :] for u in us], axis=1)
            q_cat = jnp.concatenate([qaug[u, 0:DH, :] for u in us], axis=1)
            for c in range(nch):
                tg, cn = (g, c + LAG_B) if c + LAG_B < nch else (nxt, c + LAG_B - nch)
                kb, ko = (c * KC_B) // BQ, (c * KC_B) % BQ
                dpts = dprob(tg, cn)
                ps = [pltpu.bitcast(p_s[u, c * KC_B // 2:(c + 1) * KC_B // 2, :], bf16) for u in us]
                dkv_s[kb, DH:2 * DH, ko:ko + KC_B] += _mm_nt(do_cat, jnp.concatenate(ps, axis=1))
                dss = [pltpu.bitcast(ds_s[c % (LAG_B + 1), j], bf16) for j in range(GH)]
                dkv_s[kb, 0:DH, ko:ko + KC_B] += _mm_nt(q_cat, jnp.concatenate(dss, axis=1))
                kt = kT[kb][:, ko:ko + KC_B]
                for j in range(GH):
                    dqs[j] = dqs[j] + _mm(kt, dss[j])
                dscore(tg, cn, dpts)
            for j, u in enumerate(us):
                t_s[u // H, pl.ds(pl.multiple_of((u % H) * DH, DH), DH), :] = dqs[j] * SCALE
            return _

        lax.fori_loop(0, ngrp, group, None, unroll=UNROLL_B)

    def block(b, _):
        r0 = pl.multiple_of(b * BQ, BQ)
        xn = jnp.concatenate([xnT_s[b, t] for t in range(NT_Q)], axis=1)

        qt = _mm(wqT[...], xn) * (SCALE * LOG2E)
        rows3 = lax.broadcasted_iota(i32, (H, DH, 128), 1)
        for t in range(NT_Q):
            q3 = qt[:, t * 128:(t + 1) * 128].astype(bf16).astype(f32).reshape(H, DH, 128)
            nq = jnp.sqrt(jnp.sum(q3 * q3, axis=1, keepdims=True))
            m = (nq * (kmax_s[0:1, :] * 1.01)).astype(bf16).astype(f32)
            low = jnp.where(rows3 == 0, -m, 0.0)
            qaug[t * H:(t + 1) * H] = jnp.concatenate([q3, low], axis=1).astype(bf16)

        flag_s[0] = 0

        def attempt(it, _):
            @pl.when(jnp.logical_or(it == 0, flag_s[0] == 1))
            def _():
                lmin = attn_fwd()
                bad = jnp.logical_not(jnp.min(lmin) >= L_MIN)
                flag_s[0] = jnp.where(jnp.logical_and(it == 0, bad), 1, 0)

            @pl.when(jnp.logical_and(it == 0, flag_s[0] == 1))
            def _():
                true_max_fix()
            return _

        lax.fori_loop(0, 2, attempt, None)

        pl.when(b == 0)(prep_ffn_weights)

        def dense(ts):
            c0, c1 = ts[0] * 128, (ts[-1] + 1) * 128
            rr = pl.ds(pl.multiple_of(r0 + c0, 128), c1 - c0)

            def cat(f):
                return jnp.concatenate([f(t) for t in ts], axis=1)

            def tiles(x):
                return [(t, x[:, i * 128:(i + 1) * 128]) for i, t in enumerate(ts)]

            ot_b = cat(lambda t: o_s[t * H:(t + 1) * H].reshape(D, 128)).astype(bf16)
            xt = cat(lambda t: xT_s[b, t]).astype(f32)
            ht = xt + _mm(woT[...], ot_b)
            hhat, rstd2 = _ln_stats(ht)
            hn = hhat.astype(bf16)
            g_blk = g_v[rr, :]
            gt_b = g_blk.T
            gt = gt_b.astype(f32)

            def swiglu(rows):
                gate = _mm(w1T[rows, :], hn)
                up = _mm(w3T[rows, :], hn)
                dhh = _mm(w2_v[rows, :], gt_b)
                sg = jax.nn.sigmoid(gate)
                silu = gate * sg
                hhT[rows, c0:c1] = (silu * up).astype(bf16)
                duT[rows, c0:c1] = (dhh * silu).astype(bf16)
                dgT[rows, c0:c1] = (dhh * up * (sg * (1.0 + gate * (1.0 - sg)))).astype(bf16)

            if _e('FLOOP'):
                def fchunk(i, _):
                    swiglu(pl.ds(pl.multiple_of(i * (F // 2), 16), F // 2))
                    return _
                lax.fori_loop(0, 2, fchunk, None)
            else:
                for (o, n) in F_CHUNKS:
                    swiglu(slice(o, o + n))

            hh = hhT[:, c0:c1]
            dg = dgT[:, c0:c1]
            du = duT[:, c0:c1]
            dhn = _mm(w1_v[...], dg) + _mm(w3_v[...], du)
            out_t = ht + _mm(w2T[...], hh)
            out_st[rr, :] = out_t.astype(bf16).T
            dht = gt + _ln_bwd(dhn, hhat, rstd2)
            for t, v in tiles(dht):
                dh_s[b, t] = v
            dht_b = dht.astype(bf16)
            dot = _mm(wo_v[...], dht_b)
            for t, v in tiles(dot):
                do3 = v.reshape(H, DH, 128)
                linv = linv_s[t * H:(t + 1) * H, 0:1, :]
                delta = jnp.sum(do3 * o_s[t * H:(t + 1) * H], axis=1, keepdims=True)
                hi, mid, lo = _split3(-delta * linv)
                low = jnp.where(rows3 == 0, hi, jnp.where(rows3 == 1, mid, jnp.where(rows3 == 2, lo, 0.0)))
                doaug[t * H:(t + 1) * H] = jnp.concatenate([do3 * linv, low], axis=1).astype(bf16)
            if _e('WLOOP'):
                def wchunk(i, _):
                    rows = pl.ds(pl.multiple_of(i * (F // 2), 16), F // 2)
                    dw2_a[rows, :] += _mm(hhT[rows, c0:c1], g_blk)
                    dw1_a[rows, :] += _mm_nt(dgT[rows, c0:c1], hn)
                    dw3_a[rows, :] += _mm_nt(duT[rows, c0:c1], hn)
                    return _
                lax.fori_loop(0, 2, wchunk, None)
            else:
                dw2_a[...] += _mm(hh, g_blk)
                dw1_a[...] += _mm_nt(dg, hn)
                dw3_a[...] += _mm_nt(du, hn)
            dwo_a[...] += _mm_nt(ot_b, dht_b)

        if _e('DSPLIT'):
            for t in range(NT_Q):
                dense([t])
        else:
            dense(list(range(NT_Q)))
        pltpu.make_async_copy(out_st.at[pl.ds(r0, BQ), :], out_hbm.at[pl.ds(r0, BQ), :],
                              out_sem.at[b]).start()

        @pl.when(b == NB - 1)
        def _():
            for acc, st, dst, si in ((dw1_a, dw1_st, dw1T_hbm, NO), (dw3_a, dw3_st, dw3T_hbm, NO + 1),
                                     (dw2_a, dw2_st, dw2_hbm, NO + 2), (dwo_a, dwo_st, dwo_hbm, NO + 3)):
                st[...] = acc[...].astype(bf16)
                pltpu.make_async_copy(st, dst, out_sem.at[si]).start()

        attn_bwd()
        dqt = jnp.concatenate([t_s[t] for t in range(NT_Q)], axis=1).astype(bf16)
        dwq_a[...] += _mm_nt(xn, dqt)
        dxq = _mm(wq_v[...], dqt)
        for t in range(NT_Q):
            dxq_s[b, t] = dxq[:, t * 128:(t + 1) * 128]
        return _

    lax.fori_loop(0, NB, block, None)

    st_cp = [pltpu.make_async_copy(st, dst, out_sem.at[si])
             for st, dst, si in ((dw1_st, dw1T_hbm, NO), (dw3_st, dw3T_hbm, NO + 1),
                                 (dw2_st, dw2_hbm, NO + 2), (dwo_st, dwo_hbm, NO + 3),
                                 (dwq_st, dwq_hbm, NO + 4))]
    dwq_st[...] = dwq_a[...].astype(bf16)
    st_cp[4].start()

    def dx_copy(b):
        rows = pl.ds(pl.multiple_of(b * BQ, BQ), BQ)
        return pltpu.make_async_copy(x_v.at[rows, :], dx_hbm.at[rows, :], dx_sem.at[b])

    rowsc = lax.broadcasted_iota(i32, (2 * DH, BQ), 0)

    def fin_blk(b, dwkv):
        dkv = dkv_s[b]
        dkv = jnp.where(rowsc < DH, dkv * LN2, dkv).astype(bf16)
        xn = jnp.concatenate([xnT_s[b, t] for t in range(NT_Q)], axis=1)
        dwkv = dwkv + _mm_nt(dkv, xn)
        dxkv = _mm(wkv_v[...], dkv)
        for t in range(NT_Q):
            rt = pl.multiple_of(b * BQ + t * 128, 128)
            dxn = dxq_s[b, t] + dxkv[:, t * 128:(t + 1) * 128]
            rstd = rstd_s[b, t, 0:1, :]
            xhat = (xT_s[b, t].astype(f32) - mean_s[b, t, 0:1, :]) * rstd
            dxt = dh_s[b, t] + _ln_bwd(dxn, xhat, rstd)
            x_v[pl.ds(rt, 128), :] = dxt.astype(bf16).T
        dx_copy(b).start()
        return dwkv

    dwkv = lax.fori_loop(0, NB, fin_blk, jnp.zeros((2 * DH, D), f32))
    dwkv_st[...] = dwkv.astype(bf16)
    c1 = pltpu.make_async_copy(dwkv_st.at[0:DH], dwkT_hbm, out_sem.at[NO + 6])
    c2 = pltpu.make_async_copy(dwkv_st.at[DH:2 * DH], dwvT_hbm, out_sem.at[NO + 7])
    c1.start()
    c2.start()
    for i in range(NB):
        pltpu.make_async_copy(out_st.at[pl.ds(i * BQ, BQ), :], out_hbm.at[pl.ds(i * BQ, BQ), :],
                              out_sem.at[i]).wait()
    for c in st_cp:
        c.wait()
    for b in range(NB):
        dx_copy(b).wait()
    c1.wait()
    c2.wait()


@jax.jit
def pallas_sequential_preLN__grouped_kv_mqa__glu_gated_swiglu__prompt_kernel(
    A_x: jax.Array,
    A_wq: jax.Array,
    A_wk: jax.Array,
    A_wv: jax.Array,
    A_wo: jax.Array,
    B_x: jax.Array,
    B_w1: jax.Array,
    B_w3: jax.Array,
    B_w2: jax.Array,
    grad_out: jax.Array,
):
    del B_x
    x = A_x.reshape(S, D)
    g = grad_out.reshape(S, D)
    V = pltpu.VMEM
    scratch = [
        V((S, D), bf16), V((S, D), bf16),
        V((D, D), bf16), V((D, D), bf16),
        V((D, F), bf16), V((D, F), bf16), V((F, D), bf16),
        V((2 * DH, D), bf16),
        V((D, D), bf16), V((D, D), bf16),
        V((F, D), bf16), V((F, D), bf16), V((D, F), bf16),
        V((D, 2 * DH), bf16),
        V((NB, NT_Q, D, 128), bf16), V((NB, NT_Q, D, 128), bf16),
        V((NB, NT_Q, 8, 128), f32), V((NB, NT_Q, 8, 128), f32),
        V((S, 128), f32), V((S, AUG), bf16), V((S, AUG), bf16),
        V((NB, DH, BQ), bf16), V((NB, DH, BQ), bf16), V((8, 128), f32),
        V((NU, AUG, 128), bf16), V((NU, AUG, 128), bf16),
        V((NU, S // 2, 128), i32),
        V((NU, DH, 128), f32), V((NU, 8, 128), f32),
        V((NT_Q, D, 128), f32),
        V((LAG_B + 1, GH, KC_B // 2, 128), i32),
        V((F, BQ), bf16), V((F, BQ), bf16), V((F, BQ), bf16),
        V((NB, 2 * DH, BQ), f32), V((NB, NT_Q, D, 128), f32), V((NB, NT_Q, D, 128), f32),
        V((D, D), f32), V((D, D), f32), V((F, D), f32), V((F, D), f32), V((F, D), f32),
        V((S, D), bf16), V((D, D), bf16), V((D, D), bf16),
        V((F, D), bf16), V((F, D), bf16), V((F, D), bf16),
        V((2 * DH, D), bf16),
        pltpu.SMEM((1,), i32),
        pltpu.SemaphoreType.DMA((8,)), pltpu.SemaphoreType.DMA((NB,)),
        pltpu.SemaphoreType.DMA((NO + 8,)), pltpu.SemaphoreType.DMA((NB,)),
    ]
    out_shape = [
        jax.ShapeDtypeStruct((S, D), bf16), jax.ShapeDtypeStruct((S, D), bf16),
        jax.ShapeDtypeStruct((D, D), bf16), jax.ShapeDtypeStruct((DH, D), bf16),
        jax.ShapeDtypeStruct((DH, D), bf16), jax.ShapeDtypeStruct((D, D), bf16),
        jax.ShapeDtypeStruct((F, D), bf16), jax.ShapeDtypeStruct((F, D), bf16),
        jax.ShapeDtypeStruct((F, D), bf16),
    ]
    any_spec = pl.BlockSpec(memory_space=pltpu.HBM)
    outs = pl.pallas_call(
        _kernel,
        out_shape=out_shape,
        in_specs=[any_spec] * 9,
        out_specs=[any_spec] * 9,
        scratch_shapes=scratch,
        compiler_params=pltpu.CompilerParams(vmem_limit_bytes=110 * 1024 * 1024),
        name="mqa_swiglu_fwd_bwd",
    )(x, A_wq, A_wk.T, A_wv.T, A_wo, B_w1.T, B_w3.T, B_w2, g)
    out, dx, dwq, dwkT, dwvT, dwo, dw1T, dw3T, dw2 = outs
    return (out.reshape(1, S, D), dx.reshape(1, S, D), dwq, dwkT.T, dwvT.T, dwo, dw1T.T, dw3T.T, dw2)
```

```python
import jax
import jax.numpy as jnp
from jax import lax
import jax.experimental.pallas as pl
import jax.experimental.pallas.tpu as pltpu

f32, bf16, i32 = jnp.float32, jnp.bfloat16, jnp.int32

S, D, H, DH, F = 2048, 512, 32, 16, 1376
BQ = 512
NB = S // BQ
NT_Q = BQ // 128
NO = NB
NU = NT_Q * H
GH = 4
KC_F, LAG_F, UNROLL_F = 256, 1, 4
KC_B, LAG_B, UNROLL_B = 128, 3, 4
AUG = 32
F_CHUNKS = ((0, 352), (352, 352), (704, 352), (1056, 320))
EPS = 1e-5
SCALE = DH ** -0.5
LOG2E = 1.4426950408889634
LN2 = 0.6931471805599453
L_MIN = 2.0 ** -60

NT_DIMS = (((1,), (1,)), ((), ()))


def _mm(a, b):
    return jnp.dot(a, b, preferred_element_type=f32)


def _mm_nt(a, b):
    return lax.dot_general(a, b, NT_DIMS, preferred_element_type=f32)


def _pack_rows(x):
    n = x.shape[0]
    x4 = x.reshape(n // 16, 2, 8, 128)
    a = x4[:, 0].reshape(n // 2, 128)
    b = x4[:, 1].reshape(n // 2, 128)
    return pltpu.pack_elementwise([a, b], packed_dtype=bf16)


def _halves(x):
    n = x.shape[0]
    x4 = x.reshape(n // 16, 2, 8, 128)
    return x4[:, 0].reshape(n // 2, 128), x4[:, 1].reshape(n // 2, 128)


def _unpack(x, idx):
    return pltpu.unpack_elementwise(x, index=idx, packed_dtype=bf16, unpacked_dtype=f32)


def _split3(x):
    hi = x.astype(bf16).astype(f32)
    r = x - hi
    mid = r.astype(bf16).astype(f32)
    lo = (r - mid).astype(bf16).astype(f32)
    return hi, mid, lo


def _ln_stats(xt):
    mean = jnp.mean(xt, axis=0, keepdims=True)
    xc = xt - mean
    var = jnp.mean(xc * xc, axis=0, keepdims=True)
    rstd = lax.rsqrt(var + EPS)
    return xc * rstd, rstd


def _ln_bwd(dy, xhat, rstd):
    m1 = jnp.mean(dy, axis=0, keepdims=True)
    m2 = jnp.mean(dy * xhat, axis=0, keepdims=True)
    return rstd * (dy - m1 - xhat * m2)


def _kernel(x_hbm, wq_hbm, wkT_hbm, wvT_hbm, wo_hbm, w1T_hbm, w3T_hbm, w2_hbm, g_hbm,
            out_hbm, dx_hbm, dwq_hbm, dwkT_hbm, dwvT_hbm, dwo_hbm, dw1T_hbm, dw3T_hbm, dw2_hbm,
            x_v, g_v, wq_v, wo_v, w1_v, w3_v, w2_v, wkvT,
            wqT, woT, w1T, w3T, w2T, wkv_v,
            xT_s, xnT_s, mean_s, rstd_s,
            kvrow_s, kaug, vaug, kT, vT, kmax_s,
            qaug, doaug, p_s, o_s, linv_s, t_s, ds_s,
            hhT, dgT, duT,
            dkv_s, dh_s, dxq_s,
            dwq_a, dwo_a, dw1_a, dw3_a, dw2_a,
            out_st, dwkv_st,
            flag_s, in_sem, x_sem, out_sem, dx_sem):

    dwq_st, dwo_st, dw1_st, dw3_st, dw2_st = wq_v, wo_v, w1T, w3T, w2_v

    def x_copy(b):
        rows = pl.ds(pl.multiple_of(b * BQ, BQ), BQ)
        return pltpu.make_async_copy(x_hbm.at[rows, :], x_v.at[rows, :], x_sem.at[b])

    ins = [(wq_hbm, wq_v), (wkT_hbm, wkvT.at[0:DH]), (wvT_hbm, wkvT.at[DH:2 * DH]),
           (wo_hbm, wo_v), (w1T_hbm, w1T), (w3T_hbm, w3T), (w2_hbm, w2_v), (g_hbm, g_v)]
    in_cp = [None] + [pltpu.make_async_copy(s, d, in_sem.at[i]) for i, (s, d) in enumerate(ins)]
    in_cp[2].start()
    in_cp[3].start()
    for b in range(NB):
        x_copy(b).start()
    in_cp[1].start()

    dkv_s[...] = jnp.zeros(dkv_s.shape, f32)
    flag_s[0] = 0

    in_cp[2].wait()
    in_cp[3].wait()

    wkv_pad = jnp.concatenate([wkvT[...].astype(f32), jnp.zeros((128 - 2 * DH, D), f32)], axis=0)
    wkv_v[...] = wkv_pad.T[:, 0:2 * DH].astype(bf16)

    def setup_blk(b, kn2max):
        r0 = pl.multiple_of(b * BQ, BQ)
        x_copy(b).wait()
        xtb = x_v[pl.ds(r0, BQ), :].T
        xt = xtb.astype(f32)
        mean = jnp.mean(xt, axis=0, keepdims=True)
        xc = xt - mean
        var = jnp.mean(xc * xc, axis=0, keepdims=True)
        rstd = lax.rsqrt(var + EPS)
        xn = (xc * rstd).astype(bf16)
        for t in range(NT_Q):
            sl = slice(t * 128, (t + 1) * 128)
            xT_s[b, t] = xtb[:, sl]
            xnT_s[b, t] = xn[:, sl]
            mean_s[b, t] = jnp.broadcast_to(mean[:, sl], (8, 128))
            rstd_s[b, t] = jnp.broadcast_to(rstd[:, sl], (8, 128))
        kvt = _mm(wkvT[...], xn).astype(bf16)
        kT[b] = kvt[0:DH]
        vT[b] = kvt[DH:2 * DH]
        kf = kvt[0:DH].astype(f32)
        kn2 = jnp.sum(kf * kf, axis=0, keepdims=True)
        kvpad = jnp.concatenate([kvt.astype(f32), jnp.zeros((128 - 2 * DH, BQ), f32)], axis=0)
        kvrow_s[pl.ds(r0, BQ), :] = kvpad.T
        return jnp.maximum(kn2max, kn2)

    kn2max = lax.fori_loop(0, NB, setup_blk, jnp.zeros((1, BQ), f32), unroll=2)
    kmax = jnp.sqrt(jnp.max(kn2max, axis=1, keepdims=True))
    kmax_s[...] = jnp.broadcast_to(kmax, (8, 128))

    lane = lax.broadcasted_iota(i32, (128, 128), 1)

    def perm_blk(c, _):
        r0 = pl.multiple_of(c * 256, 256)
        ev = kvrow_s[pl.ds(r0, 128, stride=2), :]
        od = kvrow_s[pl.ds(r0 + 1, 128, stride=2), :]
        for half, src in ((0, ev), (1, od)):
            ka = jnp.where(lane < DH, src, jnp.where(lane < DH + 3, 1.0, 0.0))
            vs = pltpu.roll(src, 128 - DH, 1)
            va = jnp.where(lane < DH, vs, jnp.where(lane < DH + 3, 1.0, 0.0))
            ka3 = ka.reshape(16, 8, 128)
            va3 = va.reshape(16, 8, 128)
            for i in range(16):
                t_s[0, pl.ds(16 * i + 8 * half, 8), :] = ka3[i]
                t_s[1, pl.ds(16 * i + 8 * half, 8), :] = va3[i]
        kaug[pl.ds(r0, 256), :] = t_s[0, 0:256, 0:AUG].astype(bf16)
        vaug[pl.ds(r0, 256), :] = t_s[1, 0:256, 0:AUG].astype(bf16)
        return _

    lax.fori_loop(0, S // 256, perm_blk, None, unroll=2)

    for i in (4, 5, 6, 7, 8):
        in_cp[i].start()
    in_cp[1].wait()
    wqT[...] = wq_v[...].T

    def prep_ffn_weights():
        in_cp[4].wait()
        woT[...] = wo_v[...].T
        for cp, src, dst in ((in_cp[5], w1T, w1_v), (in_cp[6], w3T, w3_v)):
            cp.wait()
            for (o, n) in ((0, 384), (384, 384), (768, 384), (1152, 224)):
                if n % 128 == 0:
                    dst[:, o:o + n] = src[o:o + n, :].T
                else:
                    blk = jnp.concatenate([src[o:o + n, :], jnp.zeros((256 - n, D), bf16)], axis=0)
                    dst[:, o:o + n] = blk.T[:, 0:n]
        in_cp[7].wait()
        for (o, n) in ((0, 384), (384, 384), (768, 384), (1152, 224)):
            if n % 128 == 0:
                w2T[:, o:o + n] = w2_v[o:o + n, :].T
            else:
                blk = jnp.concatenate([w2_v[o:o + n, :], jnp.zeros((256 - n, D), bf16)], axis=0)
                w2T[:, o:o + n] = blk.T[:, 0:n]
        in_cp[8].wait()

    rows32 = lax.broadcasted_iota(i32, (AUG, 128), 0)

    def attn_fwd():
        nch = S // KC_F
        ngrp = NU // GH

        def scores(g, c):
            kk = kaug[c * KC_F:(c + 1) * KC_F, :]
            return [_mm(kk, qaug[g * GH + j]) for j in range(GH)]

        def exps(g, c, st, ls):
            out = []
            for j in range(GH):
                e = jnp.exp2(st[j])
                out.append(ls[j] + jnp.sum(e.reshape(KC_F // 8, 8, 128), axis=0))
                p_s[g * GH + j, c * KC_F // 2:(c + 1) * KC_F // 2, :] = _pack_rows(e)
            return out

        ls0 = [jnp.zeros((8, 128), f32) for _ in range(GH)]
        for c in range(LAG_F):
            ls0 = exps(0, c, scores(0, c), ls0)

        def group(g, carry):
            ls, lmin = list(carry[0]), carry[1]
            nxt = jnp.minimum(g + 1, ngrp - 1)
            accs = [jnp.zeros((DH, 128), f32) for _ in range(GH)]
            ls_next = [jnp.zeros((8, 128), f32) for _ in range(GH)]
            for c in range(nch):
                cq = c + LAG_F
                wrap = cq >= nch
                tg, cq = (nxt, cq - nch) if wrap else (g, cq)
                st = scores(tg, cq)
                vt = vT[(c * KC_F) // BQ][:, (c * KC_F) % BQ:(c * KC_F) % BQ + KC_F]
                for j in range(GH):
                    p = pltpu.bitcast(p_s[g * GH + j, c * KC_F // 2:(c + 1) * KC_F // 2, :], bf16)
                    accs[j] = accs[j] + _mm(vt, p)
                if wrap:
                    ls_next = exps(tg, cq, st, ls_next)
                else:
                    ls = exps(tg, cq, st, ls)
            for j in range(GH):
                u = g * GH + j
                l = jnp.sum(ls[j], axis=0, keepdims=True)
                linv = 1.0 / l
                o_s[u] = accs[j] * linv
                linv_s[u] = jnp.broadcast_to(linv, (8, 128))
                lmin = jnp.minimum(lmin, l)
            return tuple(ls_next), lmin

        _, lmin = lax.fori_loop(0, ngrp, group, (tuple(ls0), jnp.full((1, 128), jnp.inf, f32)),
                                unroll=UNROLL_F)
        return lmin

    def true_max_fix():
        def unit(u, _):
            q = qaug[u]

            def chunk(c, mx):
                kk = kaug[pl.ds(pl.multiple_of(c * 256, 256), 256), :]
                st = _mm(kk, q)
                return jnp.maximum(mx, jnp.max(st.reshape(32, 8, 128), axis=0))

            mx = lax.fori_loop(0, S // 256, chunk, jnp.full((8, 128), -jnp.inf, f32))
            d = jnp.max(mx, axis=0, keepdims=True)
            qf = q.astype(f32)
            m_old = -(qf[DH:DH + 1] + qf[DH + 1:DH + 2] + qf[DH + 2:DH + 3])
            hi, mid, lo = _split3(-(m_old + d))
            new = jnp.where(rows32 == DH, hi,
                            jnp.where(rows32 == DH + 1, mid,
                                      jnp.where(rows32 == DH + 2, lo, qf)))
            qaug[u] = new.astype(bf16)
            return _

        lax.fori_loop(0, NU, unit, None)

    def attn_bwd():
        nch = S // KC_B
        ngrp = NU // GH

        def dprob(g, c):
            vv = vaug[c * KC_B:(c + 1) * KC_B, :]
            return [_mm(vv, doaug[g * GH + j]) for j in range(GH)]

        def dscore(g, c, dpts):
            for j in range(GH):
                pi = p_s[g * GH + j, c * KC_B // 2:(c + 1) * KC_B // 2, :]
                da, db = _halves(dpts[j])
                ds_s[c % (LAG_B + 1), j] = pltpu.pack_elementwise(
                    [_unpack(pi, 0) * da, _unpack(pi, 1) * db], packed_dtype=bf16)

        for c in range(LAG_B):
            dscore(0, c, dprob(0, c))

        def group(g, _):
            nxt = jnp.minimum(g + 1, ngrp - 1)
            us = [g * GH + j for j in range(GH)]
            dqs = [jnp.zeros((DH, 128), f32) for _ in range(GH)]
            do_cat = jnp.concatenate([doaug[u, 0:DH, :] for u in us], axis=1)
            q_cat = jnp.concatenate([qaug[u, 0:DH, :] for u in us], axis=1)
            for c in range(nch):
                tg, cn = (g, c + LAG_B) if c + LAG_B < nch else (nxt, c + LAG_B - nch)
                kb, ko = (c * KC_B) // BQ, (c * KC_B) % BQ
                kt = kT[kb][:, ko:ko + KC_B]
                dpts = dprob(tg, cn)
                ps = [pltpu.bitcast(p_s[u, c * KC_B // 2:(c + 1) * KC_B // 2, :], bf16) for u in us]
                dkv_s[kb, DH:2 * DH, ko:ko + KC_B] += _mm_nt(do_cat, jnp.concatenate(ps, axis=1))
                dss = [pltpu.bitcast(ds_s[c % (LAG_B + 1), j], bf16) for j in range(GH)]
                dkv_s[kb, 0:DH, ko:ko + KC_B] += _mm_nt(q_cat, jnp.concatenate(dss, axis=1))
                for j in range(GH):
                    dqs[j] = dqs[j] + _mm(kt, dss[j])
                dscore(tg, cn, dpts)
            for j, u in enumerate(us):
                t_s[u // H, pl.ds(pl.multiple_of((u % H) * DH, DH), DH), :] = dqs[j] * SCALE
            return _

        lax.fori_loop(0, ngrp, group, None, unroll=UNROLL_B)

    def block(b, _):
        r0 = pl.multiple_of(b * BQ, BQ)
        xn = jnp.concatenate([xnT_s[b, t] for t in range(NT_Q)], axis=1)

        def accumulate(acc, val):
            acc[...] = jnp.where(b == 0, 0.0, acc[...]) + val

        qt = _mm(wqT[...], xn) * (SCALE * LOG2E)
        rows3 = lax.broadcasted_iota(i32, (H, DH, 128), 1)
        for t in range(NT_Q):
            q3 = qt[:, t * 128:(t + 1) * 128].astype(bf16).astype(f32).reshape(H, DH, 128)
            nq = jnp.sqrt(jnp.sum(q3 * q3, axis=1, keepdims=True))
            m = (nq * (kmax_s[0:1, :] * 1.01)).astype(bf16).astype(f32)
            low = jnp.where(rows3 == 0, -m, 0.0)
            qaug[t * H:(t + 1) * H] = jnp.concatenate([q3, low], axis=1).astype(bf16)

        flag_s[0] = 0

        def attempt(it, _):
            @pl.when(jnp.logical_or(it == 0, flag_s[0] == 1))
            def _():
                lmin = attn_fwd()
                bad = jnp.logical_not(jnp.min(lmin) >= L_MIN)
                flag_s[0] = jnp.where(jnp.logical_and(it == 0, bad), 1, 0)

            @pl.when(jnp.logical_and(it == 0, flag_s[0] == 1))
            def _():
                true_max_fix()
            return _

        lax.fori_loop(0, 2, attempt, None)

        pl.when(b == 0)(prep_ffn_weights)

        def dense(ts):
            c0, c1 = ts[0] * 128, (ts[-1] + 1) * 128
            rr = pl.ds(pl.multiple_of(r0 + c0, 128), c1 - c0)

            def cat(f):
                return jnp.concatenate([f(t) for t in ts], axis=1)

            def tiles(x):
                return [(t, x[:, i * 128:(i + 1) * 128]) for i, t in enumerate(ts)]

            g_blk = g_v[rr, :]
            gt_b = g_blk.T
            gt = gt_b.astype(f32)
            ot_b = cat(lambda t: o_s[t * H:(t + 1) * H].reshape(D, 128)).astype(bf16)
            xt = cat(lambda t: xT_s[b, t]).astype(f32)
            ht = xt + _mm(woT[...], ot_b)
            early = {o: _mm(w2_v[o:o + n, :], gt_b) for (o, n) in F_CHUNKS[:1]}
            hhat, rstd2 = _ln_stats(ht)
            hn = hhat.astype(bf16)

            for (o, n) in F_CHUNKS:
                gate = _mm(w1T[o:o + n, :], hn)
                up = _mm(w3T[o:o + n, :], hn)
                dhh = early[o] if o in early else _mm(w2_v[o:o + n, :], gt_b)
                sg = jax.nn.sigmoid(gate)
                silu = gate * sg
                hhT[o:o + n, c0:c1] = (silu * up).astype(bf16)
                duT[o:o + n, c0:c1] = (dhh * silu).astype(bf16)
                dgT[o:o + n, c0:c1] = (dhh * up * (sg * (1.0 + gate * (1.0 - sg)))).astype(bf16)

            hh = hhT[:, c0:c1]
            dg = dgT[:, c0:c1]
            du = duT[:, c0:c1]
            dhn = _mm(w1_v[...], dg) + _mm(w3_v[...], du)
            out_t = ht + _mm(w2T[...], hh)
            out_st[rr, :] = out_t.astype(bf16).T
            dht = gt + _ln_bwd(dhn, hhat, rstd2)
            for t, v in tiles(dht):
                dh_s[b, t] = v
            dht_b = dht.astype(bf16)
            dot = _mm(wo_v[...], dht_b)
            for t, v in tiles(dot):
                do3 = v.reshape(H, DH, 128)
                linv = linv_s[t * H:(t + 1) * H, 0:1, :]
                delta = jnp.sum(do3 * o_s[t * H:(t + 1) * H], axis=1, keepdims=True)
                hi, mid, lo = _split3(-delta * linv)
                low = jnp.where(rows3 == 0, hi, jnp.where(rows3 == 1, mid, jnp.where(rows3 == 2, lo, 0.0)))
                doaug[t * H:(t + 1) * H] = jnp.concatenate([do3 * linv, low], axis=1).astype(bf16)
            accumulate(dw2_a, _mm(hh, g_blk))
            accumulate(dw1_a, _mm_nt(dg, hn))
            accumulate(dw3_a, _mm_nt(du, hn))
            accumulate(dwo_a, _mm_nt(ot_b, dht_b))

        dense(list(range(NT_Q)))
        pltpu.make_async_copy(out_st.at[pl.ds(r0, BQ), :], out_hbm.at[pl.ds(r0, BQ), :],
                              out_sem.at[b]).start()

        @pl.when(b == NB - 1)
        def _():
            for acc, st, dst, si in ((dw1_a, dw1_st, dw1T_hbm, NO), (dw3_a, dw3_st, dw3T_hbm, NO + 1),
                                     (dw2_a, dw2_st, dw2_hbm, NO + 2), (dwo_a, dwo_st, dwo_hbm, NO + 3)):
                st[...] = acc[...].astype(bf16)
                pltpu.make_async_copy(st, dst, out_sem.at[si]).start()

        attn_bwd()
        dqt = jnp.concatenate([t_s[t] for t in range(NT_Q)], axis=1).astype(bf16)
        accumulate(dwq_a, _mm_nt(xn, dqt))
        dxq = _mm(wq_v[...], dqt)
        for t in range(NT_Q):
            dxq_s[b, t] = dxq[:, t * 128:(t + 1) * 128]
        return _

    lax.fori_loop(0, NB, block, None)

    st_cp = [pltpu.make_async_copy(st, dst, out_sem.at[si])
             for st, dst, si in ((dw1_st, dw1T_hbm, NO), (dw3_st, dw3T_hbm, NO + 1),
                                 (dw2_st, dw2_hbm, NO + 2), (dwo_st, dwo_hbm, NO + 3),
                                 (dwq_st, dwq_hbm, NO + 4))]
    dwq_st[...] = dwq_a[...].astype(bf16)
    st_cp[4].start()

    def dx_copy(i):
        rows = pl.ds(pl.multiple_of(i * 128, 128), 128)
        return pltpu.make_async_copy(x_v.at[rows, :], dx_hbm.at[rows, :], dx_sem.at[i])

    rowsc = lax.broadcasted_iota(i32, (2 * DH, BQ), 0)

    def fin_blk(b, dwkv):
        dkv = dkv_s[b]
        dkv = jnp.where(rowsc < DH, dkv * LN2, dkv).astype(bf16)
        xn = jnp.concatenate([xnT_s[b, t] for t in range(NT_Q)], axis=1)
        dwkv = dwkv + _mm_nt(dkv, xn)
        dxkv = _mm(wkv_v[...], dkv)
        for t in range(NT_Q):
            rt = pl.multiple_of(b * BQ + t * 128, 128)
            dxn = dxq_s[b, t] + dxkv[:, t * 128:(t + 1) * 128]
            rstd = rstd_s[b, t, 0:1, :]
            xhat = (xT_s[b, t].astype(f32) - mean_s[b, t, 0:1, :]) * rstd
            dxt = dh_s[b, t] + _ln_bwd(dxn, xhat, rstd)
            x_v[pl.ds(rt, 128), :] = dxt.astype(bf16).T
            dx_copy(b * NT_Q + t).start()
        return dwkv

    dwkv = lax.fori_loop(0, NB, fin_blk, jnp.zeros((2 * DH, D), f32))
    dwkv_st[...] = dwkv.astype(bf16)
    c1 = pltpu.make_async_copy(dwkv_st.at[0:DH], dwkT_hbm, out_sem.at[NO + 6])
    c2 = pltpu.make_async_copy(dwkv_st.at[DH:2 * DH], dwvT_hbm, out_sem.at[NO + 7])
    c1.start()
    c2.start()
    for i in range(NB):
        pltpu.make_async_copy(out_st.at[pl.ds(i * BQ, BQ), :], out_hbm.at[pl.ds(i * BQ, BQ), :],
                              out_sem.at[i]).wait()
    for c in st_cp:
        c.wait()
    for i in range(NB * NT_Q):
        dx_copy(i).wait()
    c1.wait()
    c2.wait()


@jax.jit
def pallas_sequential_preLN__grouped_kv_mqa__glu_gated_swiglu__prompt_kernel(
    A_x: jax.Array,
    A_wq: jax.Array,
    A_wk: jax.Array,
    A_wv: jax.Array,
    A_wo: jax.Array,
    B_x: jax.Array,
    B_w1: jax.Array,
    B_w3: jax.Array,
    B_w2: jax.Array,
    grad_out: jax.Array,
):
    del B_x
    x = A_x.reshape(S, D)
    g = grad_out.reshape(S, D)
    V = pltpu.VMEM
    scratch = [
        V((S, D), bf16), V((S, D), bf16),
        V((D, D), bf16), V((D, D), bf16),
        V((D, F), bf16), V((D, F), bf16), V((F, D), bf16),
        V((2 * DH, D), bf16),
        V((D, D), bf16), V((D, D), bf16),
        V((F, D), bf16), V((F, D), bf16), V((D, F), bf16),
        V((D, 2 * DH), bf16),
        V((NB, NT_Q, D, 128), bf16), V((NB, NT_Q, D, 128), bf16),
        V((NB, NT_Q, 8, 128), f32), V((NB, NT_Q, 8, 128), f32),
        V((S, 128), f32), V((S, AUG), bf16), V((S, AUG), bf16),
        V((NB, DH, BQ), bf16), V((NB, DH, BQ), bf16), V((8, 128), f32),
        V((NU, AUG, 128), bf16), V((NU, AUG, 128), bf16),
        V((NU, S // 2, 128), i32),
        V((NU, DH, 128), f32), V((NU, 8, 128), f32),
        V((NT_Q, D, 128), f32),
        V((LAG_B + 1, GH, KC_B // 2, 128), i32),
        V((F, BQ), bf16), V((F, BQ), bf16), V((F, BQ), bf16),
        V((NB, 2 * DH, BQ), f32), V((NB, NT_Q, D, 128), f32), V((NB, NT_Q, D, 128), f32),
        V((D, D), f32), V((D, D), f32), V((F, D), f32), V((F, D), f32), V((F, D), f32),
        V((S, D), bf16),
        V((2 * DH, D), bf16),
        pltpu.SMEM((1,), i32),
        pltpu.SemaphoreType.DMA((8,)), pltpu.SemaphoreType.DMA((NB,)),
        pltpu.SemaphoreType.DMA((NO + 8,)), pltpu.SemaphoreType.DMA((NB * NT_Q,)),
    ]
    out_shape = [
        jax.ShapeDtypeStruct((S, D), bf16), jax.ShapeDtypeStruct((S, D), bf16),
        jax.ShapeDtypeStruct((D, D), bf16), jax.ShapeDtypeStruct((DH, D), bf16),
        jax.ShapeDtypeStruct((DH, D), bf16), jax.ShapeDtypeStruct((D, D), bf16),
        jax.ShapeDtypeStruct((F, D), bf16), jax.ShapeDtypeStruct((F, D), bf16),
        jax.ShapeDtypeStruct((F, D), bf16),
    ]
    any_spec = pl.BlockSpec(memory_space=pltpu.HBM)
    outs = pl.pallas_call(
        _kernel,
        out_shape=out_shape,
        in_specs=[any_spec] * 9,
        out_specs=[any_spec] * 9,
        scratch_shapes=scratch,
        compiler_params=pltpu.CompilerParams(vmem_limit_bytes=126 * 1024 * 1024),
        name="mqa_swiglu_fwd_bwd",
    )(x, A_wq, A_wk.T, A_wv.T, A_wo, B_w1.T, B_w3.T, B_w2, g)
    out, dx, dwq, dwkT, dwvT, dwo, dw1T, dw3T, dw2 = outs
    return (out.reshape(1, S, D), dx.reshape(1, S, D), dwq, dwkT.T, dwvT.T, dwo, dw1T.T, dw3T.T, dw2)
```
